```python
import os as _os
_os.environ.setdefault("JAX_PLATFORMS", "cpu")
import jax
import jax.numpy as jnp

def _softmax(x, axis=-1):
    return jax.nn.softmax(x, axis=axis)
def _gelu(x):
    return jax.nn.gelu(x, approximate=True)
def _silu(x):
    return jax.nn.silu(x)
def _sigmoid(x):
    return jax.nn.sigmoid(x)
def _layernorm(x, axis=-1, eps=1e-5):
    m = jnp.mean(x, axis=axis, keepdims=True)
    v = jnp.var(x, axis=axis, keepdims=True)
    return (x - m) / jnp.sqrt(v + eps)
def _scatter_add(tgt, idx, src, axis=0):
    return tgt.at[idx].add(src)
def _segment_sum(src, seg, n):
    return jax.ops.segment_sum(src, seg, n)
class _Rng:
    def __init__(self, key):
        self._k = key
    def _next(self):
        self._k, sub = jax.random.split(self._k)
        return sub
    def normal(self, shape):
        return jax.random.normal(self._next(), shape, dtype=jnp.bfloat16)
    def randint(self, lo, hi, shape):
        return jax.random.randint(self._next(), shape, lo, hi, dtype=jnp.int32)
    def uniform(self, shape, lo=0.0, hi=1.0):
        return jax.random.uniform(self._next(), shape, jnp.bfloat16, lo, hi)
    def permutation(self, n):
        return jax.random.permutation(self._next(), n)


kernel_name = 'sequential_preLN__softmax_full_mha__mixer_channel_mlp__prompt'

def setup_inputs():
    _rng = _Rng(jax.random.key(int.from_bytes(__import__("os").urandom(4), "little")))
    _w = (lambda a: (lambda t: t.astype(jnp.bfloat16) if jnp.issubdtype(t.dtype, jnp.floating) else t)(jnp.asarray(a)))
    def _A_setup():
        B, S, D = 1, 2048, 1024
        return {
            "x": _w((lambda *s: _rng.normal(s) * 0.05)(B, S, D)),
            "wqkv": _w((lambda *s: _rng.normal(s) * 0.05)(D, 3 * D)),
            "wo": _w((lambda *s: _rng.normal(s) * 0.05)(D, D)),
        }
    _A_in = _A_setup()

    def _B_setup():
        B, S, D, F = 1, 2048, 1024, 3584
        return {
            "x": _w((lambda *s: _rng.normal(s) * 0.05)(B, S, D)),
            "w1": _w((lambda *s: _rng.normal(s) * 0.8)(D, F) * (D ** -0.5)),
            "b1": _w((lambda *s: _rng.normal(s) * 0.8)(F)),
            "w2": _w((lambda *s: _rng.normal(s) * 0.8)(F, D) * (F ** -0.5)),
            "b2": _w((lambda *s: _rng.normal(s) * 0.05)(D)),
        }
    _B_in = _B_setup()

    return {
        "A_x": _A_in["x"],
        "A_wqkv": _A_in["wqkv"],
        "A_wo": _A_in["wo"],
        "B_x": _B_in["x"],
        "B_w1": _B_in["w1"],
        "B_b1": _B_in["b1"],
        "B_w2": _B_in["w2"],
        "B_b2": _B_in["b2"],
    }

def reference(A_x, A_wqkv, A_wo, B_x, B_w1, B_b1, B_w2, B_b2):
    def _A_ref(x, wqkv, wo):
        B, S, D = x.shape
        H = 32; Dh = D // H
        qkv = (lambda x, *d: x.transpose(*d))((x @ wqkv).reshape(B, S, 3, H, Dh), 2, 0, 3, 1, 4)
        q, k, v = qkv[0], qkv[1], qkv[2]
        scale = Dh ** -0.5
        scores = jnp.einsum("bhqd,bhkd->bhqk", q, k) * scale
        p = _softmax(scores, axis=-1)
        o = jnp.einsum("bhqk,bhkd->bhqd", p, v)
        return (lambda x, *d: x.transpose(*d))(o, 0, 2, 1, 3).reshape(B, S, D) @ wo

    def _B_ref(x, w1, b1, w2, b2):
        y = _layernorm(x, axis=-1)
        h = _gelu(jnp.einsum("bsd,df->bsf", y, w1) + b1)
        return jnp.einsum("bsf,fd->bsd", h, w2) + b2

    x = A_x
    h = x + _A_ref(_layernorm(x, axis=-1), A_wqkv, A_wo)
    h2 = h + _B_ref(_layernorm(h, axis=-1), B_w1, B_b1, B_w2, B_b2)
    return h2
```

```python
import functools
import numpy as np
import jax
import jax.numpy as jnp
from jax import lax
from jax.experimental import pallas as pl
from jax.experimental.pallas import tpu as pltpu

S, D, H, DH, F = 2048, 1024, 32, 32, 3584
G = D // 128
HPG = 128 // DH
EPS = 1e-5
LOG2E = float(np.log2(np.e))
f32, bf16 = jnp.float32, jnp.bfloat16


def _ln(x):
    m = jnp.mean(x, axis=-1, keepdims=True)
    xc = x - m
    v = jnp.mean(xc * xc, axis=-1, keepdims=True)
    return xc * lax.rsqrt(v + EPS)


def _gelu(u):
    c0 = float(np.sqrt(2.0 / np.pi))
    c1 = c0 * 0.044715
    t = jnp.tanh(u * (c0 + c1 * (u * u)))
    hu = 0.5 * u
    return hu + hu * t


def make(TQ=256, CK=128, U=8, lag=4, nch=1, nbuf=4, TM=128, FC=512, apos=0, scopes=False, skip=(), flags=None):
    NQ = S // TQ
    NC = S // CK
    CPB = TQ // CK
    NH = NQ * H
    NM = S // TM
    NF = F // FC
    MPB = TQ // TM
    import contextlib
    scope = (lambda n: jax.named_scope(n)) if scopes else (lambda n: contextlib.nullcontext())

    def kern(x_hbm, wqkv_hbm, wo_hbm, w1_hbm, b1_hbm, w2_hbm, b2_hbm, out_hbm,
             x_v, wqkv_v, wo_v, w1_v, b1_v, w2_v, b2_v,
             k_s, qT_s, vT_s, oT_s, y_s, h_s, out_v, sem_in, sem_out, *bufs):
        def xcp(b):
            return pltpu.make_async_copy(x_hbm.at[pl.ds(b * TQ, TQ)], x_v.at[pl.ds(b * TQ, TQ)], sem_in.at[b])
        def wcp(j):
            return pltpu.make_async_copy(wqkv_hbm.at[:, pl.ds(j * D, D)], wqkv_v.at[j], sem_in.at[NQ + j])
        rest = [pltpu.make_async_copy(s_, d_, sem_in.at[NQ + 3 + n]) for n, (s_, d_) in enumerate(
            [(wo_hbm, wo_v), (w1_hbm, w1_v), (b1_hbm, b1_v), (w2_hbm, w2_v), (b2_hbm, b2_v)])]
        xcp(0).start(); wcp(0).start(); xcp(1).start(); wcp(1).start(); wcp(2).start()
        for b in range(2, NQ):
            xcp(b).start()
        for c in rest:
            c.start()

        def ln1(b):
            r0 = pl.multiple_of(b * TQ, TQ)
            y_s[pl.ds(r0, TQ), :] = _ln(x_v[pl.ds(r0, TQ), :].astype(f32)).astype(bf16)

        def qkv(b, first=False):
            r0 = pl.multiple_of(b * TQ, TQ)
            y = y_s[pl.ds(r0, TQ), :]
            if first: wcp(0).wait()
            q = jnp.dot(y, wqkv_v[0], preferred_element_type=f32) * (DH ** -0.5 * LOG2E)
            qT_s[b] = q.T.astype(bf16)
            if first: wcp(1).wait()
            v = jnp.dot(y, wqkv_v[2 if not first else 1], preferred_element_type=f32)
            if first:
                k = v.astype(bf16)
                wcp(2).wait()
                v = jnp.dot(y, wqkv_v[2], preferred_element_type=f32)
                vT_s[b] = v.T.astype(bf16)
            else:
                vT_s[b] = v.T.astype(bf16)
                k = jnp.dot(y, wqkv_v[1], preferred_element_type=f32).astype(bf16)
            for g in range(G):
                k_s[g, pl.ds(r0, TQ), :] = k[:, g * 128:(g + 1) * 128]

        if 1 not in skip:
            with scope("ph1a"):
                xcp(0).wait()
                ln1(0)
                xcp(1).wait()
                qkv(0, True)
                ln1(1)
                for b in range(2, NQ):
                    xcp(b).wait()
            def ph1(b, _):
                qkv(b)
                ln1(jnp.minimum(b + 1, NQ - 1))
                return None
            with scope("ph1b"):
                lax.fori_loop(1, NQ, ph1, None)
        else:
            for b in range(NQ): xcp(b).wait()
            for j in range(3): wcp(j).wait()

        def idx(hh):
            return hh >> 5, pl.multiple_of((hh & (H - 1)) * DH, DH)

        def qpad(hh, j):
            i, r = idx(hh)
            qh = qT_s[i, pl.ds(r, DH), :]
            parts = []
            if j > 0: parts.append(jnp.zeros((j * DH, TQ), bf16))
            parts.append(qh)
            if j < HPG - 1: parts.append(jnp.zeros(((HPG - 1 - j) * DH, TQ), bf16))
            return jnp.concatenate(parts, axis=0)

        def red(op, acc, x, rev):
            n = x.shape[0] // 8
            acc = list(acc) if acc is not None else [None] * nch
            for r in (range(n - 1, -1, -1) if rev else range(n)):
                y = x[r * 8:(r + 1) * 8]
                a = acc[r % nch]
                acc[r % nch] = y if a is None else op(a, y)
            return acc

        def p1(hh, qp, c, scr, m, z):
            g = (hh & (H - 1)) >> 2
            s = jnp.dot(k_s[g, c * CK:(c + 1) * CK, :], qp, preferred_element_type=f32)
            scr[z, c * CK:(c + 1) * CK, :] = s
            return red(jnp.maximum, m, s, False)

        def p2(hh, c, scr, mb, l, acc, z):
            _, r = idx(hh)
            s = scr[z, c * CK:(c + 1) * CK, :]
            p = jnp.exp2(s.reshape(CK // 8, 8, TQ) - mb[None]).reshape(CK, TQ)
            l = red(jnp.add, l, p, True)
            cb, cc = divmod(c, CPB)
            vt = vT_s[cb, pl.ds(r, DH), cc * CK:(cc + 1) * CK]
            pv = jnp.dot(vt, p.astype(bf16), preferred_element_type=f32)
            return l, (pv if acc is None else acc + pv)

        def fin(hh, l, acc):
            i, r = idx(hh)
            ls = jnp.sum(functools.reduce(jnp.add, l), axis=0, keepdims=True)
            o = (acc * (1.0 / ls)).astype(bf16)
            for sub in range(MPB):
                oT_s[i * MPB + sub, pl.ds(r, DH), :] = o[:, sub * TM:(sub + 1) * TM]

        def bc(m):
            return jnp.broadcast_to(jnp.max(functools.reduce(jnp.maximum, m), axis=0, keepdims=True), (8, TQ))

        def run_slots(base, n0, n1, m, mnext, zs, zl, p1_hi):
            qp = mb = l = acc = None
            for n in range(n0, n1):
                if n < p1_hi:
                    h1, c1 = divmod(n, NC)
                    if qp is None or c1 == 0:
                        qp = qpad(base + h1, h1 % HPG)
                    m = p1(base + h1, qp, c1, bufs[h1 % nbuf], None if c1 == 0 else m, zs)
                    if c1 == NC - 1:
                        mnew = bc(m); m = None
                    else:
                        mnew = None
                n2 = n - NC - lag
                if n2 >= 0:
                    h2, c2 = divmod(n2, NC)
                    if c2 == 0:
                        mb, l, acc = mnext, None, None
                    l, acc = p2(base + h2, c2, bufs[h2 % nbuf], mb, l, acc, zl)
                    if c2 == NC - 1:
                        fin(base + h2, l, acc)
                if n < p1_hi and mnew is not None:
                    mnext = mnew
            return m, mnext

        if 2 not in skip:
            BIG = 1 << 30
            with scope("att_pro"):
                st = run_slots(0, 0, NC + lag, None, None, 0, 0, BIG)
            def body(t, st):
                return run_slots(t * U, NC + lag, NC + lag + U * NC, st[0], st[1], t >> 10, t >> 11, BIG)
            with scope("att_loop"):
                st = lax.fori_loop(0, NH // U - 1, body, st)
            with scope("att_epi"):
                z = pl.program_id(0) if False else 0
                run_slots(NH - U, NC + lag, NC + lag + U * NC, st[0], st[1], 0, 0, U * NC)

        for c in rest:
            c.wait()

        def ocp(b):
            return pltpu.make_async_copy(out_v.at[pl.ds(b * TM, TM)], out_hbm.at[pl.ds(b * TM, TM)], sem_out.at[b])

        def stageA(b):
            r0 = pl.multiple_of(b * TM, TM)
            o = oT_s[b].astype(f32).T.astype(bf16)
            h = x_v[pl.ds(r0, TM), :].astype(f32) + jnp.dot(o, wo_v[...], preferred_element_type=f32)
            h_s[pl.ds(r0, TM), :] = h + b2_v[...].astype(f32)
            y_s[pl.ds(r0, TM), :] = _ln(h).astype(bf16)

        def stageB(b, mid=None):
            r0 = pl.multiple_of(b * TM, TM)
            y = y_s[pl.ds(r0, TM), :]
            acc = h_s[pl.ds(r0, TM), :]
            for c in range(NF):
                if c == apos and mid is not None:
                    mid()
                u = jnp.dot(y, w1_v[:, c * FC:(c + 1) * FC], preferred_element_type=f32) + b1_v[:, c * FC:(c + 1) * FC].astype(f32)
                acc = acc + jnp.dot(_gelu(u).astype(bf16), w2_v[c * FC:(c + 1) * FC, :], preferred_element_type=f32)
            if apos >= NF and mid is not None:
                mid()
            out_v[pl.ds(r0, TM), :] = acc.astype(bf16)

        if 3 not in skip:
            with scope("ph3_pro"):
                stageA(0)
            def ph3(b, _):
                stageB(b, lambda: stageA(b + 1))
                ocp(b).start()
            with scope("ph3_loop"):
                lax.fori_loop(0, NM - 1, ph3, None)
            with scope("ph3_epi"):
                stageB(NM - 1)
                ocp(NM - 1).start()
                for b in range(NM):
                    ocp(b).wait()

    def f(A_x, A_wqkv, A_wo, B_x, B_w1, B_b1, B_w2, B_b2):
        del B_x
        any_spec = pl.BlockSpec(memory_space=pl.ANY)
        out = pl.pallas_call(
            kern, name="fused",
            out_shape=jax.ShapeDtypeStruct((S, D), bf16),
            in_specs=[any_spec] * 7, out_specs=any_spec,
            scratch_shapes=[
                pltpu.VMEM((S, D), bf16), pltpu.VMEM((3, D, D), bf16), pltpu.VMEM((D, D), bf16),
                pltpu.VMEM((D, F), bf16), pltpu.VMEM((1, F), bf16), pltpu.VMEM((F, D), bf16), pltpu.VMEM((1, D), bf16),
                pltpu.VMEM((G, S, 128), bf16), pltpu.VMEM((NQ, D, TQ), bf16), pltpu.VMEM((NQ, D, TQ), bf16),
                pltpu.VMEM((NM, D, TM), bf16),
                pltpu.VMEM((S, D), bf16), pltpu.VMEM((S, D), f32), pltpu.VMEM((S, D), bf16),
                pltpu.SemaphoreType.DMA((NQ + 8,)), pltpu.SemaphoreType.DMA((NM,)),
            ] + [pltpu.VMEM((1, S, TQ), f32)] * nbuf,
            compiler_params=pltpu.CompilerParams(vmem_limit_bytes=110 * 1024 * 1024, flags=flags),
        )(A_x.reshape(S, D), A_wqkv, A_wo, B_w1, B_b1.reshape(1, F), B_w2, B_b2.reshape(1, D))
        return out.reshape(1, S, D)
    return f


_impl = make(TM=128,FC=896,apos=2)


@jax.jit
def pallas_sequential_preLN__softmax_full_mha__mixer_channel_mlp__prompt_kernel(
    A_x, A_wqkv, A_wo, B_x, B_w1, B_b1, B_w2, B_b2
):
    return _impl(A_x, A_wqkv, A_wo, B_x, B_w1, B_b1, B_w2, B_b2)
```

```python
import contextlib
import functools
import numpy as np
import jax
import jax.numpy as jnp
from jax import lax
from jax.experimental import pallas as pl
from jax.experimental.pallas import tpu as pltpu

S, D, H, DH, F = 2048, 1024, 32, 32, 3584
G = D // 128
HPG = 128 // DH
EPS = 1e-5
LOG2E = float(np.log2(np.e))
f32, bf16, u32 = jnp.float32, jnp.bfloat16, jnp.uint32
VM = pltpu.VMEM


def _ln(x):
    m = jnp.mean(x, axis=-1, keepdims=True)
    xc = x - m
    v = jnp.mean(xc * xc, axis=-1, keepdims=True)
    return xc * lax.rsqrt(v + EPS)


def _gelu(u):
    c0 = float(np.sqrt(2.0 / np.pi))
    c1 = c0 * 0.044715
    t = jnp.tanh(u * (c0 + c1 * (u * u)))
    hu = 0.5 * u
    return hu + hu * t


def _quads(x):
    n = len(x) // 2
    return ([r[:n] for r in x[:n]], [r[n:] for r in x[:n]], [r[:n] for r in x[n:]], [r[n:] for r in x[n:]])


def _add(a, b):
    return [[p + q for p, q in zip(ra, rb)] for ra, rb in zip(a, b)]


def _sub(a, b):
    return [[p - q for p, q in zip(ra, rb)] for ra, rb in zip(a, b)]


def _enc_a(x):
    if len(x) == 1:
        return [x[0][0]]
    a11, a12, a21, a22 = _quads(x)
    ops = [_add(a11, a22), _add(a21, a22), a11, a22, _add(a11, a12), _sub(a21, a11), _sub(a12, a22)]
    return [z for o in ops for z in _enc_a(o)]


def _enc_b(x):
    if len(x) == 1:
        return [x[0][0]]
    b11, b12, b21, b22 = _quads(x)
    ops = [_add(b11, b22), b11, _sub(b12, b22), _sub(b21, b11), b22, _add(b11, b12), _add(b21, b22)]
    return [z for o in ops for z in _enc_b(o)]


_B_TERMS = (((0, 0, 1), (1, 1, 1)), ((0, 0, 1),), ((0, 1, 1), (1, 1, -1)), ((1, 0, 1), (0, 0, -1)), ((1, 1, 1),),
            ((0, 0, 1), (0, 1, 1)), ((1, 0, 1), (1, 1, 1)))


def _dec(prod, lo, n):
    if n == 1:
        return [[prod(lo)]]
    s7 = n // 7
    m1, m2, m3, m4, m5, m6, m7 = [_dec(prod, lo + i * s7, s7) for i in range(7)]
    c11 = _add(_sub(_add(m1, m4), m5), m7)
    c12 = _add(m3, m5)
    c21 = _add(m2, m4)
    c22 = _add(_add(_sub(m1, m2), m3), m6)
    return [a + b for a, b in zip(c11, c12)] + [a + b for a, b in zip(c21, c22)]


def _blocks(x, n):
    r, c = x.shape[0] // n, x.shape[1] // n
    return [[x[i * r:(i + 1) * r, j * c:(j + 1) * c] for j in range(n)] for i in range(n)]


def _join(c):
    return jnp.concatenate([jnp.concatenate(r, axis=1) for r in c], axis=0)


def _upk(x):
    return pltpu.bitcast(x, bf16)


def _mm(a, b):
    return jnp.dot(a, b, preferred_element_type=f32)


def _mult(i, n):
    return i * n if isinstance(i, int) else pl.multiple_of(i * n, n)


def _halves(x):
    w = pltpu.bitcast(x, u32)
    return [pltpu.unpack_elementwise(w, index=p, packed_dtype=bf16, unpacked_dtype=f32) for p in range(2)]


def _pack(lo, hi):
    return pltpu.pack_elementwise([lo, hi], packed_dtype=bf16)


def make(CK=128, U=16, lag=4, nbuf=4, FC=128, WCH=(256, 256, 512, 512, 512, 512, 512), pin1=1, pin0=1, ahead=2, peel=1,
         wo_at="att", epi=0, scopes=False, flags=None):
    TQ = TM = 256
    NQ = S // TQ
    NC = S // CK
    CPB = TQ // CK
    NH = NQ * H
    NIT = NH // U
    HD = D // 2
    QM, QD, QF = TM // 4, D // 4, F // 4
    NP = QF // 128
    assert NP == NQ - 1
    NW = len(WCH)
    WO_ = [sum(WCH[:j]) for j in range(NW + 1)]
    MCOL = (0, 2 * D, D)
    scope = (lambda n: jax.named_scope(n)) if scopes else (lambda n: contextlib.nullcontext())

    def kern(x_hbm, wqkv_hbm, wo_hbm, w1_hbm, b1_hbm, w2_hbm, b2_hbm, out_hbm,
             x_v, b1_s, b2_s, wos, w1s, w2s, oT_s, zero_s, sem_x, sem_w, sem_p, sem_r, sem_out):
        zero_s[0] = 0
        pl.run_scoped(
            functools.partial(attention, x_hbm, wqkv_hbm, wo_hbm, w1_hbm, b1_hbm, w2_hbm, b2_hbm,
                              x_v, b1_s, b2_s, wos, w1s, w2s, oT_s, zero_s, sem_x, sem_w, sem_p, sem_r),
            VM((D + 16, D), bf16), VM((F,), bf16), VM((D,), bf16),
            VM((G, S, 128), bf16), VM((NQ, D, TQ), bf16), VM((NQ, D, TQ), bf16))
        pl.run_scoped(
            functools.partial(mlp, out_hbm, x_v, b1_s, b2_s, wos, w1s, w2s, oT_s, sem_out),
            VM((TM, D), f32), VM((49, QM, QD), bf16), VM((2, TM, D), bf16))

    def attention(x_hbm, wqkv_hbm, wo_hbm, w1_hbm, b1_hbm, w2_hbm, b2_hbm,
                  x_v, b1_s, b2_s, wos, w1s, w2s, oT_s, zero_s, sem_x, sem_w, sem_p, sem_r,
                  wo_v, b1_v, b2_v, k_s, qT_s, vT_s):
        rest = [pltpu.make_async_copy(s_, d_, sem_r.at[n]) for n, (s_, d_) in enumerate(
            [(b1_hbm, b1_v), (b2_hbm, b2_v), (wo_hbm, wo_v.at[pl.ds(0, D)])])]

        def prep2(load, store, i1):
            acc = [None, None]
            for qh, ch, sg in _B_TERMS[i1]:
                raw = [[_halves(load(2 * qh + q, 2 * ch + c)) for c in range(2)] for q in range(2)]
                for p in range(2):
                    u = [[t[p] for t in row] for row in raw]
                    acc[p] = u if acc[p] is None else (_add if sg > 0 else _sub)(acc[p], u)
            for i2, (lo, hi) in enumerate(zip(_enc_b(acc[0]), _enc_b(acc[1]))):
                store(i1 * 7 + i2, _pack(lo, hi))

        def phase1(wqkv_v, wqs, xa_s, w1_v, w2_v):
            def xcp(b):
                return pltpu.make_async_copy(x_hbm.at[pl.ds(b * TQ, TQ)], x_v.at[pl.ds(b * TQ, TQ)], sem_x.at[b])

            def wcol(j):
                return MCOL[WO_[j] // D] + WO_[j] % D

            def wcp(j):
                sl = pl.ds(wcol(j), WCH[j])
                return pltpu.make_async_copy(wqkv_hbm.at[:, sl], wqkv_v.at[pl.ds(0, D), sl], sem_w.at[j])

            def pcps(p):
                c = _mult(p, 128)
                return ([pltpu.make_async_copy(w1_hbm.at[:, pl.ds(n * QF + c, 128)], w1_v.at[p, n, pl.ds(0, D)], sem_p.at[p])
                         for n in range(4)]
                        + [pltpu.make_async_copy(w2_hbm.at[pl.ds(n * QF + c, 128)], w2_v.at[p, n, pl.ds(0, 128)], sem_p.at[p])
                           for n in range(4)])

            queue = [[xcp(0)]] + [[wcp(j)] for j in range(NW)] + [[xcp(1), xcp(2)], pcps(0)]

            def advance(n=1):
                for _ in range(n):
                    if queue:
                        for c in queue.pop(0):
                            c.start()
            advance(1 + ahead)

            def ln1(b):
                return _ln(x_v[pl.ds(_mult(b, TQ), TQ), :].astype(f32))

            def enc1(b):
                for i, o in enumerate(_enc_a(_blocks(ln1(b), 2))):
                    xa_s[i] = o.astype(bf16)

            def put_q(b, q):
                qT_s[b] = (q * (DH ** -0.5 * LOG2E)).T.astype(bf16)

            def put_v(b, v):
                vT_s[b] = v.T.astype(bf16)

            def put_k(b, k):
                k = k.astype(bf16)
                for g in range(G):
                    k_s[g, pl.ds(_mult(b, TQ), TQ), :] = k[:, g * 128:(g + 1) * 128]
            puts = (put_q, put_v, put_k)

            def prep1(mi, rg, j):
                raw = [[_halves(wqkv_v[q * HD + rg * 16:q * HD + (rg + 1) * 16,
                                       MCOL[mi] + c * HD + j * 128:MCOL[mi] + c * HD + (j + 1) * 128])
                        for c in range(2)] for q in range(2)]
                lo, hi = [_enc_b([[t[p] for t in row] for row in raw]) for p in range(2)]
                for i in range(7):
                    wqs[i, rg * 8:(rg + 1) * 8, mi * HD + j * 128:mi * HD + (j + 1) * 128] = _pack(lo[i], hi[i])

            def spread(r, jobs, pin):
                nt = (r.shape[0] // 16) * (r.shape[1] // 128)
                for e, job in enumerate(jobs):
                    t = e * nt // len(jobs)
                    jj, aa = divmod(t, r.shape[0] // 16)
                    pin(e, r[aa * 16:(aa + 1) * 16, jj * 128:(jj + 1) * 128])
                    job()

            def qkv_first():
                xcp(0).wait()
                y = ln1(0).astype(bf16)
                parts, later, jobs = [], [], []
                for j in range(NW):
                    wcp(j).wait()
                    advance(1 if j < NW - 1 else len(queue))
                    if j == NW - 1:
                        xcp(1).wait()
                    z = zero_s[0]
                    r = _mm(y, wqkv_v[:D, wcol(j):wcol(j) + WCH[j]])
                    parts.append(r)
                    for fn in later:
                        fn()
                    later = []
                    if WO_[j + 1] % D == 0:
                        mi = WO_[j + 1] // D - 1
                        later.append(functools.partial(puts[mi], 0, jnp.concatenate(parts, axis=1)))
                        parts = []
                        jobs += [functools.partial(prep1, mi, rg, c) for rg in range(HD // 16) for c in range(HD // 128)]

                    def pin(e, v):
                        if pin0:
                            wqkv_v[pl.ds(pl.multiple_of(D + z * 16, 16), 16), :128] = v.astype(bf16)
                    n = len(jobs) if j == NW - 1 else min(len(jobs), WCH[j] // 8)
                    spread(r, jobs[:n], pin)
                    jobs = jobs[n:]
                for fn in later:
                    fn()
                enc1(1)

            def qkv(b):
                p = b - 1
                for c in pcps(p):
                    c.wait()

                @pl.when(b + 1 < NQ)
                def _():
                    xcp(b + 1).wait()
                    for c in pcps(b):
                        c.start()

                @pl.when(b + 2 < NQ)
                def _():
                    xcp(b + 2).start()

                @pl.when(b + 2 == NQ)
                def _():
                    for c in rest:
                        c.start()
                xa = [xa_s[i] for i in range(7)]
                enc1(jnp.minimum(b + 1, NQ - 1))
                z = b >> 10
                jobs, pins = [], []
                for rg in range(QD // 16):
                    def ld1(q, c, rg=rg):
                        return w1_v[p, c, q * QD + rg * 16:q * QD + (rg + 1) * 16, :]

                    def st1(i, v, rg=rg):
                        w1s[i, p, rg * 8:(rg + 1) * 8, :] = v
                    jobs += [functools.partial(prep2, ld1, st1, i1) for i1 in range(7)]
                    pins += [w1_v] * 7
                for rg in range(128 // 16):
                    for j in range(QD // 128):
                        def ld2(q, c, rg=rg, j=j):
                            return w2_v[p, q, rg * 16:(rg + 1) * 16, c * QD + j * 128:c * QD + (j + 1) * 128]

                        def st2(i, v, rg=rg, j=j):
                            w2s[i, pl.ds(pl.multiple_of(p * 64 + rg * 8, 8), 8), j * 128:(j + 1) * 128] = v
                        jobs += [functools.partial(prep2, ld2, st2, i1) for i1 in range(7)]
                        pins += [w2_v] * 7
                per = -(-len(jobs) // 20)

                def prod(mi, i):
                    r = _mm(xa[i], _upk(wqs[i, :, mi * HD:(mi + 1) * HD]))
                    k0 = (mi * 7 + i) * per

                    def pin(e, v):
                        if pin1:
                            ref = pins[k0 + e]
                            ref[z, 0, ref.shape[2] - 16:, :128] = v.astype(bf16)
                    if jobs[k0:k0 + per]:
                        spread(r, jobs[k0:k0 + per], pin)
                    return r
                for mi in range(3):
                    puts[mi](b, _join(_dec(functools.partial(prod, mi), 0, 7)))

            with scope("ph1a"):
                qkv_first()
            with scope("ph1b"):
                lax.fori_loop(1, NQ, lambda b, _: qkv(b), None)

        pl.run_scoped(phase1, VM((D + 16, 3 * D), bf16), VM((7, HD // 2, 3 * HD), u32), VM((7, TQ // 2, HD), bf16),
                      VM((NP, 4, D + 16, 128), bf16), VM((NP, 4, 128 + 16, D), bf16))

        for c in rest:
            c.wait()
        b1_s[...] = jnp.broadcast_to(b1_v[...].astype(f32).reshape(1, F), (8, F))
        b2_s[...] = jnp.broadcast_to(b2_v[...].astype(f32).reshape(1, D), (8, D))

        def wo_jobs(rg):
            jobs = []
            for j in range(QD // 128):
                def ld(q, c, j=j):
                    return wo_v[pl.ds(pl.multiple_of(q * QD + rg * 16, 16), 16), c * QD + j * 128:c * QD + (j + 1) * 128]

                def st(i, v, j=j):
                    wos[i, pl.ds(_mult(rg, 8), 8), j * 128:(j + 1) * 128] = v
                jobs += [functools.partial(prep2, ld, st, i1) for i1 in range(7)]
            return jobs

        if wo_at == "solo":
            def solo(t, _):
                for job in wo_jobs(t):
                    job()
            with scope("prep"):
                lax.fori_loop(0, QD // 16, solo, None)

        def idx(hh):
            return hh >> 5, _mult(hh & (H - 1), DH)

        def qpad(hh, j):
            i, r = idx(hh)
            qh = qT_s[i, pl.ds(r, DH), :]
            parts = []
            if j > 0:
                parts.append(jnp.zeros((j * DH, TQ), bf16))
            parts.append(qh)
            if j < HPG - 1:
                parts.append(jnp.zeros(((HPG - 1 - j) * DH, TQ), bf16))
            return jnp.concatenate(parts, axis=0)

        def red(op, acc, x, rev):
            n = x.shape[0] // 8
            for r in (range(n - 1, -1, -1) if rev else range(n)):
                y = x[r * 8:(r + 1) * 8]
                acc = y if acc is None else op(acc, y)
            return acc

        def p1(hh, qp, c, scr, m, z):
            g = (hh & (H - 1)) >> 2
            s = _mm(k_s[g, c * CK:(c + 1) * CK, :], qp)
            scr[z, c * CK:(c + 1) * CK, :] = s
            return red(jnp.maximum, m, s, False), s

        def p2(hh, c, scr, mb, l, acc, z):
            _, r = idx(hh)
            s = scr[z, c * CK:(c + 1) * CK, :]
            p = jnp.exp2(s.reshape(CK // 8, 8, TQ) - mb[None]).reshape(CK, TQ)
            l = red(jnp.add, l, p, True)
            cb, cc = divmod(c, CPB)
            vt = vT_s[cb, pl.ds(r, DH), cc * CK:(cc + 1) * CK]
            pv = _mm(vt, p.astype(bf16))
            return l, (pv if acc is None else acc + pv)

        def fin(hh, l, acc):
            i, r = idx(hh)
            ls = jnp.sum(l, axis=0, keepdims=True)
            oT_s[i, pl.ds(r, DH), :] = (acc * (1.0 / ls)).astype(bf16)

        def run_slots(bufs, base, n0, n1, m, mnext, zs, zl, p1_hi, jobs=()):
            qp = mb = l = acc = None
            step = (n1 - n0 - 8) // max(len(jobs), 1)
            for n in range(n0, n1):
                mnew = None
                if n < p1_hi:
                    h1, c1 = divmod(n, NC)
                    hh = base + h1
                    if h1 >= U:
                        hh = jnp.minimum(hh, NH - HPG + h1 % HPG)
                    if qp is None or c1 == 0:
                        qp = qpad(hh, h1 % HPG)
                    m, s = p1(hh, qp, c1, bufs[h1 % nbuf], None if c1 == 0 else m, zs)
                    if c1 == NC - 1:
                        mnew = jnp.broadcast_to(jnp.max(m, axis=0, keepdims=True), (8, TQ))
                        m = None
                    e, rem = divmod(n - n0 - 4, step)
                    if rem == 0 and 0 <= e < len(jobs):
                        wo_v[pl.ds(pl.multiple_of(D + zs * 16, 16), 16), :128] = s[:16, :128].astype(bf16)
                        jobs[e]()
                n2 = n - NC - lag
                if n2 >= 0:
                    h2, c2 = divmod(n2, NC)
                    if c2 == 0:
                        mb, l, acc = mnext, None, None
                    l, acc = p2(base + h2, c2, bufs[h2 % nbuf], mb, l, acc, zl)
                    if c2 == NC - 1:
                        fin(base + h2, l, acc)
                if mnew is not None:
                    mnext = mnew
            return m, mnext

        def phase2(*bufs):
            BIG = 1 << 30
            with scope("att_pro"):
                st = run_slots(bufs, 0, 0, NC + lag, None, None, 0, 0, BIG)
            nloop = NIT - 1 if epi else NIT

            def body(t, st):
                jobs = []
                if wo_at == "att":
                    per = -(-(QD // 16) // nloop)
                    for e in range(per):
                        jobs += wo_jobs(jnp.minimum(t * per, QD // 16 - per) + e)
                return run_slots(bufs, t * U, NC + lag, NC + lag + U * NC, st[0], st[1], t >> 10, t >> 11, BIG, jobs)
            with scope("att_loop"):
                st = lax.fori_loop(0, nloop, body, st)
            if epi:
                with scope("att_epi"):
                    z = zero_s[0]
                    run_slots(bufs, NH - U, NC + lag, NC + lag + U * NC, st[0], st[1], z, z + z, U * NC)
        pl.run_scoped(phase2, *([VM((1, S, TQ), f32)] * nbuf))

    def mlp(out_hbm, x_v, b1_s, b2_s, wos, w1s, w2s, oT_s, sem_out, hB_s, ya_s, out_v):
        def ocp(b, slot):
            return pltpu.make_async_copy(out_v.at[slot], out_hbm.at[pl.ds(_mult(b, TM), TM)], sem_out.at[slot])

        def stageA(b):
            oa = [z.astype(bf16) for z in _enc_a(_blocks(oT_s[b].astype(f32).T, 4))]
            a = _join(_dec(lambda i: _mm(oa[i], _upk(wos[i])), 0, 49))
            h = x_v[pl.ds(_mult(b, TM), TM), :].astype(f32) + a
            hB_s[...] = (h.reshape(TM // 8, 8, D) + b2_s[...][None]).reshape(TM, D)
            for i, o in enumerate(_enc_a(_blocks(_ln(h), 4))):
                ya_s[i] = o.astype(bf16)

        def stageB(b, nxt):
            ya = [ya_s[i] for i in range(49)]
            hres = hB_s[...]
            gas = []
            for c in range(QF // 128):
                u = _dec(lambda i: _mm(ya[i], _upk(w1s[i, c])), 0, 49)
                g = [[_gelu((u[r][n].reshape(QM // 8, 8, 128)
                             + b1_s[:, n * QF + c * 128:n * QF + (c + 1) * 128][None]).reshape(QM, 128))
                      for n in range(4)] for r in range(4)]
                gas.append([z.astype(bf16) for z in _enc_a(g)])
            if nxt is not None:
                stageA(nxt)
            c = _dec(lambda i: _mm(jnp.concatenate([ga[i] for ga in gas], axis=1), _upk(w2s[i])), 0, 49)
            return (hres + _join(c)).astype(bf16)

        with scope("ph3_pro"):
            stageA(0)

        def ph3(b, _):
            slot = b & 1

            @pl.when(b >= 2)
            def _():
                ocp(b - 2, slot).wait()
            out_v[slot] = stageB(b, jnp.minimum(b + 1, NQ - 1))
            ocp(b, slot).start()
        with scope("ph3_loop"):
            lax.fori_loop(0, NQ - 1 if peel else NQ, ph3, None)
        with scope("ph3_epi"):
            if peel:
                ocp(NQ - 3, (NQ - 3) % 2).wait()
                out_v[(NQ - 1) % 2] = stageB(NQ - 1, None)
                ocp(NQ - 1, (NQ - 1) % 2).start()
            ocp(NQ - 2, (NQ - 2) % 2).wait()
            ocp(NQ - 1, (NQ - 1) % 2).wait()

    def f(A_x, A_wqkv, A_wo, B_x, B_w1, B_b1, B_w2, B_b2):
        del B_x
        any_spec = pl.BlockSpec(memory_space=pl.ANY)
        out = pl.pallas_call(
            kern, name="fused",
            out_shape=jax.ShapeDtypeStruct((S, D), bf16),
            in_specs=[any_spec] * 7, out_specs=any_spec,
            scratch_shapes=[
                VM((S, D), bf16), VM((8, F), f32), VM((8, D), f32),
                VM((49, QD // 2, QD), u32), VM((49, NP, QD // 2, 128), u32), VM((49, QF // 2, QD), u32),
                VM((NQ, D, TQ), bf16), pltpu.SMEM((1,), jnp.int32),
                pltpu.SemaphoreType.DMA((NQ,)), pltpu.SemaphoreType.DMA((NW,)), pltpu.SemaphoreType.DMA((NP,)),
                pltpu.SemaphoreType.DMA((3,)), pltpu.SemaphoreType.DMA((2,)),
            ],
            compiler_params=pltpu.CompilerParams(vmem_limit_bytes=127 * 1024 * 1024, flags=flags),
        )(A_x.reshape(S, D), A_wqkv, A_wo, B_w1, B_b1, B_w2, B_b2)
        return out.reshape(1, S, D)
    return f


_impl = make(ahead=3)


@jax.jit
def pallas_sequential_preLN__softmax_full_mha__mixer_channel_mlp__prompt_kernel(
    A_x, A_wqkv, A_wo, B_x, B_w1, B_b1, B_w2, B_b2
):
    return _impl(A_x, A_wqkv, A_wo, B_x, B_w1, B_b1, B_w2, B_b2)
```

```python
import functools

import jax
import jax.numpy as jnp
import numpy as np
from jax import lax
from jax.experimental import pallas as pl
from jax.experimental.pallas import tpu as pltpu

S, D, H, DH, F = 2048, 1024, 32, 32, 3584
EPS = 1e-5
Q_SCALE = float(DH ** -0.5 * np.log2(np.e))
GELU_C0 = float(np.sqrt(2.0 / np.pi))
GELU_C1 = GELU_C0 * 0.044715

T = 256
NB = S // T
G = D // 128
HPG = 128 // DH
CK = 128
NC = S // CK
NH = NB * H
U = 16
LAG = 4
NSB = 4
HD = D // 2
QT, QD, QF = T // 4, D // 4, F // 4
NP = QF // 128
W_CHUNKS = (256, 256, 256, 256, 512, 512, 512, 512)
W_ORDER = (0, 2 * D, D)
X1_CHUNK = 6
assert NP == NB - 1 and sum(W_CHUNKS) == 3 * D

f32, bf16, u32 = jnp.float32, jnp.bfloat16, jnp.uint32
VMEM = pltpu.VMEM


def _layernorm(x):
    xc = x - jnp.mean(x, axis=-1, keepdims=True)
    return xc * lax.rsqrt(jnp.mean(xc * xc, axis=-1, keepdims=True) + EPS)


def _gelu(u):
    hu = 0.5 * u
    return hu + hu * jnp.tanh(u * (GELU_C0 + GELU_C1 * (u * u)))


def _mm(a, b):
    return jnp.dot(a, b, preferred_element_type=f32)


def _times(i, n):
    return i * n if isinstance(i, int) else pl.multiple_of(i * n, n)


def _add_rows(x, row):
    return (x.reshape(x.shape[0] // 8, 8, x.shape[1]) + row[None]).reshape(x.shape)


def _pack(x):
    return pltpu.bitcast(x.astype(bf16), u32)


def _unpack(x):
    return pltpu.bitcast(x, bf16)


_A_TERMS = (((0, 0, 1), (1, 1, 1)), ((1, 0, 1), (1, 1, 1)), ((0, 0, 1),), ((1, 1, 1),),
            ((0, 0, 1), (0, 1, 1)), ((1, 0, 1), (0, 0, -1)), ((0, 1, 1), (1, 1, -1)))
_B_TERMS = (((0, 0, 1), (1, 1, 1)), ((0, 0, 1),), ((0, 1, 1), (1, 1, -1)), ((1, 0, 1), (0, 0, -1)),
            ((1, 1, 1),), ((0, 0, 1), (0, 1, 1)), ((1, 0, 1), (1, 1, 1)))


def _add(a, b):
    return [[p + q for p, q in zip(ra, rb)] for ra, rb in zip(a, b)]


def _sub(a, b):
    return [[p - q for p, q in zip(ra, rb)] for ra, rb in zip(a, b)]


def _combine(terms, quadrant):
    acc = None
    for rh, ch, sign in terms:
        q = quadrant(rh, ch)
        acc = q if acc is None else (_add if sign > 0 else _sub)(acc, q)
    return acc


def _operands(all_terms, x):
    if len(x) == 1:
        return [x[0][0]]
    n = len(x) // 2
    quadrant = lambda rh, ch: [row[ch * n:(ch + 1) * n] for row in x[rh * n:(rh + 1) * n]]
    return [o for terms in all_terms for o in _operands(all_terms, _combine(terms, quadrant))]


def _results(product, first, n):
    if n == 1:
        return [[product(first)]]
    m1, m2, m3, m4, m5, m6, m7 = [_results(product, first + i * (n // 7), n // 7) for i in range(7)]
    c11 = _add(_sub(_add(m1, m4), m5), m7)
    c12 = _add(m3, m5)
    c21 = _add(m2, m4)
    c22 = _add(_add(_sub(m1, m2), m3), m6)
    return [a + b for a, b in zip(c11, c12)] + [a + b for a, b in zip(c21, c22)]


def _join(grid):
    return jnp.concatenate([jnp.concatenate(row, axis=1) for row in grid], axis=0)


def _second_level(all_terms, load, store, i1):
    quadrant = lambda rh, ch: [[load(2 * rh + r, 2 * ch + c) for c in range(2)] for r in range(2)]
    for i2, o in enumerate(_operands(all_terms, _combine(all_terms[i1], quadrant))):
        store(i1 * 7 + i2, o)


def _park(ref, z, r):
    if len(ref.shape) == 2:
        ref[pl.ds(pl.multiple_of(ref.shape[0] - 16 + z * 16, 16), 16), :128] = r[:16, :128].astype(bf16)
    elif len(ref.shape) == 4:
        ref[z, 0, ref.shape[2] - 16:, :128] = r[:16, :128].astype(bf16)
    elif ref.dtype == f32:
        ref[z, ref.shape[1] - 8:, :128] = r[:8, :128]
    else:
        ref[ref.shape[0] - 1 + z, :16, :128] = r[:16, :128].astype(bf16)


def _spread(r, jobs, z):
    row_tiles = r.shape[0] // 16
    tiles = row_tiles * (r.shape[1] // 128)
    for e, (ref, fn) in enumerate(jobs):
        j, a = divmod(e * tiles // len(jobs), row_tiles)
        _park(ref, z, r[a * 16:(a + 1) * 16, j * 128:(j + 1) * 128])
        fn()


def _interleave(few, many):
    step = len(many) // len(few)
    return [t for e, job in enumerate(few) for t in [job] + many[e * step:(e + 1) * step]] + many[len(few) * step:]


def _qkv_phase(x_hbm, wqkv_hbm, w1_hbm, w2_hbm, x_v, w1s, w2s, k_s, qT_s, vT_s, zero_s, sem_x, sem_w, sem_p,
               late_copies, wqkv_v, wqs, xa_s, y_s, w1_v, w2_v):
    bounds = [sum(W_CHUNKS[:j]) for j in range(len(W_CHUNKS) + 1)]

    def x_copy(b):
        return pltpu.make_async_copy(x_hbm.at[pl.ds(b * T, T)], x_v.at[pl.ds(b * T, T)], sem_x.at[b])

    def w_col(j):
        return W_ORDER[bounds[j] // D] + bounds[j] % D

    def w_copy(j):
        cols = pl.ds(w_col(j), W_CHUNKS[j])
        return pltpu.make_async_copy(wqkv_hbm.at[:, cols], wqkv_v.at[pl.ds(0, D), cols], sem_w.at[j])

    def part_copies(p):
        c = _times(p, 128)
        return ([pltpu.make_async_copy(w1_hbm.at[:, pl.ds(n * QF + c, 128)], w1_v.at[p, n, pl.ds(0, D)], sem_p.at[p])
                 for n in range(4)]
                + [pltpu.make_async_copy(w2_hbm.at[pl.ds(n * QF + c, 128)], w2_v.at[p, n, pl.ds(0, 128)], sem_p.at[p])
                   for n in range(4)])

    queue = ([[x_copy(0)]]
             + [[w_copy(j)] + ([x_copy(1)] if j == X1_CHUNK else []) for j in range(len(W_CHUNKS))]
             + [[x_copy(2)], part_copies(0)])

    def advance(n):
        for _ in range(min(n, len(queue))):
            for c in queue.pop(0):
                c.start()

    def x_jobs(b):
        def norm(rg):
            rows = x_v[pl.ds(_times(b * (T // 16) + rg, 16), 16), :]
            y_s[0, rg * 16:(rg + 1) * 16, :] = _layernorm(rows.astype(f32))

        def encode(rg, j):
            grid = [[y_s[0, r * (T // 2) + rg * 16:r * (T // 2) + (rg + 1) * 16, c * HD + j * 128:c * HD + (j + 1) * 128]
                     for c in range(2)] for r in range(2)]
            for i, o in enumerate(_operands(_A_TERMS, grid)):
                xa_s[i, rg * 16:(rg + 1) * 16, j * 128:(j + 1) * 128] = o.astype(bf16)

        return ([(x_v, functools.partial(norm, rg)) for rg in range(T // 16)]
                + [(y_s, functools.partial(encode, rg, j)) for rg in range(T // 32) for j in range(HD // 128)])

    def wqkv_jobs(m):
        def encode(rg, j):
            grid = [[wqkv_v[r * HD + rg * 16:r * HD + (rg + 1) * 16,
                            W_ORDER[m] + c * HD + j * 128:W_ORDER[m] + c * HD + (j + 1) * 128].astype(f32)
                     for c in range(2)] for r in range(2)]
            for i, o in enumerate(_operands(_B_TERMS, grid)):
                wqs[i, rg * 8:(rg + 1) * 8, m * HD + j * 128:m * HD + (j + 1) * 128] = _pack(o)

        return [(wqkv_v, functools.partial(encode, rg, j)) for rg in range(HD // 16) for j in range(HD // 128)]

    def mlp_weight_jobs(p):
        jobs = []
        for rg in range(QD // 16):
            def load1(r, c, rg=rg):
                return w1_v[p, c, r * QD + rg * 16:r * QD + (rg + 1) * 16, :].astype(f32)

            def store1(i, o, rg=rg):
                w1s[i, p, rg * 8:(rg + 1) * 8, :] = _pack(o)

            jobs += [(w1_v, functools.partial(_second_level, _B_TERMS, load1, store1, i1)) for i1 in range(7)]
        for rg in range(128 // 16):
            for j in range(QD // 128):
                def load2(r, c, rg=rg, j=j):
                    return w2_v[p, r, rg * 16:(rg + 1) * 16, c * QD + j * 128:c * QD + (j + 1) * 128].astype(f32)

                def store2(i, o, rg=rg, j=j):
                    w2s[i, pl.ds(_times(p * 8 + rg, 8), 8), j * 128:(j + 1) * 128] = _pack(o)

                jobs += [(w2_v, functools.partial(_second_level, _B_TERMS, load2, store2, i1)) for i1 in range(7)]
        return jobs

    def put_q(b, q):
        qT_s[b] = (q * Q_SCALE).T.astype(bf16)

    def put_v(b, v):
        vT_s[b] = v.T.astype(bf16)

    def put_k(b, k):
        k = k.astype(bf16)
        for g in range(G):
            k_s[g, pl.ds(_times(b, T), T), :] = k[:, g * 128:(g + 1) * 128]

    puts = (put_q, put_v, put_k)

    advance(2)
    x_copy(0).wait()
    advance(2)
    y = _layernorm(x_v[:T, :].astype(f32)).astype(bf16)
    parts, deferred, backlog = [], [], []
    for j, width in enumerate(W_CHUNKS):
        last = j == len(W_CHUNKS) - 1
        w_copy(j).wait()
        advance(len(queue) if last else 1)
        if j == X1_CHUNK:
            x_copy(1).wait()
        lo = _mm(y[:, :HD], wqkv_v[:HD, w_col(j):w_col(j) + width])
        hi = _mm(y[:, HD:], wqkv_v[HD:D, w_col(j):w_col(j) + width])
        parts.append(lo + hi)
        for fn in deferred:
            fn()
        deferred = []
        if bounds[j + 1] % D == 0:
            m = bounds[j + 1] // D - 1
            deferred.append(functools.partial(puts[m], 0, jnp.concatenate(parts, axis=1)))
            parts = []
            backlog += wqkv_jobs(m)
        if j == X1_CHUNK:
            backlog = _interleave(x_jobs(1), backlog)
        n = len(backlog) if last else min(len(backlog), width * 3 // 16)
        z = zero_s[0]
        _spread(lo, backlog[:n * 5 // 9], z)
        _spread(hi[:, :width * 3 // 4 // 128 * 128], backlog[n * 5 // 9:n], z)
        backlog = backlog[n:]
    for fn in deferred:
        fn()

    def block(b, _):
        for c in part_copies(b - 1):
            c.wait()

        @pl.when(b + 1 < NB)
        def _():
            x_copy(b + 1).wait()
            for c in part_copies(b):
                c.start()

        @pl.when(b + 2 < NB)
        def _():
            x_copy(b + 2).start()

        @pl.when(b + 2 == NB)
        def _():
            for c in late_copies:
                c.start()

        xa = [xa_s[i] for i in range(7)]
        jobs = _interleave(x_jobs(jnp.minimum(b + 1, NB - 1)), mlp_weight_jobs(b - 1))
        per = -(-len(jobs) // 21)

        def product(i):
            r = _mm(xa[i % 7], _unpack(wqs[i % 7, :, i // 7 * HD:(i // 7 + 1) * HD]))
            _spread(r, jobs[i * per:(i + 1) * per], b >> 10)
            return r

        for m in range(3):
            puts[m](b, _join(_results(product, m * 7, 7)))

    lax.fori_loop(1, NB, block, None)


def _attention_phase(k_s, qT_s, vT_s, oT_s, wo_v, wos, zero_s, mlp_input, *score_bufs):
    def locate(pair):
        return pair >> 5, _times(pair & (H - 1), DH)

    def padded_q(pair, j):
        i, row = locate(pair)
        above = [jnp.zeros((j * DH, T), bf16)] if j > 0 else []
        below = [jnp.zeros(((HPG - 1 - j) * DH, T), bf16)] if j < HPG - 1 else []
        return jnp.concatenate(above + [qT_s[i, pl.ds(row, DH), :]] + below, axis=0)

    def fold(op, acc, x, order):
        for r in order:
            acc = x[r * 8:(r + 1) * 8] if acc is None else op(acc, x[r * 8:(r + 1) * 8])
        return acc

    def scores(pair, q, c, buf, m, z):
        s = _mm(k_s[(pair & (H - 1)) >> 2, c * CK:(c + 1) * CK, :], q)
        buf[z, c * CK:(c + 1) * CK, :] = s
        return fold(jnp.maximum, m, s, range(CK // 8)), s

    def weigh(pair, c, buf, m, denom, acc, z):
        s = buf[z, c * CK:(c + 1) * CK, :]
        p = jnp.exp2(s.reshape(CK // 8, 8, T) - m[None]).reshape(CK, T)
        denom = fold(jnp.add, denom, p, range(CK // 8 - 1, -1, -1))
        kb, kc = divmod(c, T // CK)
        pv = _mm(vT_s[kb, pl.ds(locate(pair)[1], DH), kc * CK:(kc + 1) * CK], p.astype(bf16))
        return denom, (pv if acc is None else acc + pv)

    def finish(pair, denom, acc):
        i, row = locate(pair)
        oT_s[i, pl.ds(row, DH), :] = (acc * (1.0 / jnp.sum(denom, axis=0, keepdims=True))).astype(bf16)

    def run(base, first, stop, m, ready, z_store, z_load, scores_stop, jobs=()):
        q = row_max = denom = acc = None
        for n in range(first, stop):
            done = None
            if n < scores_stop:
                h, c = divmod(n, NC)
                if q is None or c == 0:
                    q = padded_q(base + h, h % HPG)
                m, s = scores(base + h, q, c, score_bufs[h % NSB], None if c == 0 else m, z_store)
                if c == NC - 1:
                    done, m = jnp.broadcast_to(jnp.max(m, axis=0, keepdims=True), (8, T)), None
                for slot, ref, fn in jobs:
                    if slot == n - first:
                        if ref is not None:
                            _park(ref, z_store, s)
                        fn()
            if n >= NC + LAG:
                h, c = divmod(n - NC - LAG, NC)
                if c == 0:
                    row_max, denom, acc = ready, None, None
                denom, acc = weigh(base + h, c, score_bufs[h % NSB], row_max, denom, acc, z_load)
                if c == NC - 1:
                    finish(base + h, denom, acc)
            if done is not None:
                ready = done
        return m, ready

    def wo_jobs(rg):
        jobs = []
        for j in range(QD // 128):
            def load(r, c, j=j):
                rows = pl.ds(_times(r * (QD // 16) + rg, 16), 16)
                return wo_v[rows, c * QD + j * 128:c * QD + (j + 1) * 128].astype(f32)

            def store(i, o, j=j):
                wos[i, pl.ds(_times(rg, 8), 8), j * 128:(j + 1) * 128] = _pack(o)

            jobs += [(wo_v, functools.partial(_second_level, _B_TERMS, load, store, i1)) for i1 in range(7)]
        return jobs

    def pace(jobs, first, last):
        return [(first + e * (last - first) // len(jobs), ref, fn) for e, (ref, fn) in enumerate(jobs)]

    first, stop, never = NC + LAG, NC + LAG + U * NC, 1 << 30
    state = run(0, 0, first, None, None, 0, 0, never)

    def body(t, state):
        return run(t * U, first, stop, *state, t >> 10, t >> 11, never, pace(wo_jobs(t), 4, U * NC - 4))

    state = lax.fori_loop(0, NH // U - 1, body, state)

    o_jobs, out_proj, y_jobs = mlp_input
    jobs = (pace(wo_jobs(NH // U - 1), 2, 30) + pace(o_jobs(0), 30, 110)
            + [(110, None, functools.partial(out_proj, 0))] + pace(y_jobs(), 120, 230))
    z = zero_s[0]
    run(NH - U, first, stop, *state, z, z + z, U * NC, jobs)


def _mlp_input(x_v, wos, oT_s, h_s, t_s, oa_s, ya_s):
    def encode_jobs(dst):
        jobs = []
        for i1 in range(7):
            for rg in range(QT // 16):
                for j in range(QD // 128):
                    def load(r, c, rg=rg, j=j):
                        return t_s[0, r * QT + rg * 16:r * QT + (rg + 1) * 16, c * QD + j * 128:c * QD + (j + 1) * 128]

                    def store(i, o, rg=rg, j=j):
                        dst[i, rg * 16:(rg + 1) * 16, j * 128:(j + 1) * 128] = o.astype(bf16)

                    jobs.append((t_s, functools.partial(_second_level, _A_TERMS, load, store, i1)))
        return jobs

    def o_jobs(b):
        def transpose(g, j):
            tile = oT_s[b, g * 128:(g + 1) * 128, j * 128:(j + 1) * 128]
            t_s[0, j * 128:(j + 1) * 128, g * 128:(g + 1) * 128] = tile.astype(f32).T

        return ([(oT_s, functools.partial(transpose, g, j)) for g in range(G) for j in range(T // 128)]
                + encode_jobs(oa_s))

    def out_proj(b):
        attn = _results(lambda i: _mm(oa_s[i], _unpack(wos[i])), 0, 49)
        for r in range(4):
            for c in range(4):
                x = x_v[pl.ds(_times(b * 4 + r, QT), QT), c * QD:(c + 1) * QD]
                h_s[0, r * QT:(r + 1) * QT, c * QD:(c + 1) * QD] = x.astype(f32) + attn[r][c]

    def y_jobs():
        def norm(rg):
            t_s[0, rg * 16:(rg + 1) * 16, :] = _layernorm(h_s[0, rg * 16:(rg + 1) * 16, :])

        return [(h_s, functools.partial(norm, rg)) for rg in range(T // 16)] + encode_jobs(ya_s)

    return o_jobs, out_proj, y_jobs


def _mlp_phase(out_hbm, b1_s, b2_s, w1s, w2s, h_s, ya_s, sem_out, mlp_input, out_v):
    o_jobs, out_proj, y_jobs = mlp_input

    def out_copy(b, slot):
        return pltpu.make_async_copy(out_v.at[slot], out_hbm.at[pl.ds(_times(b, T), T)], sem_out.at[slot])

    def block(b, more):
        def paced(product, n, jobs):
            def run(i):
                r = product(i)
                for e, (ref, fn) in enumerate(jobs):
                    if e * n // len(jobs) == i:
                        _park(ref, b >> 10, r)
                        fn()
                return r
            return run

        ya = [ya_s[i] for i in range(49)]
        h = h_s[0, :T]
        up = paced(lambda i: _mm(ya[i % 49], _unpack(w1s[i % 49, i // 49])), 49 * NP, o_jobs(b + 1) if more else [])
        hidden = []
        for p in range(NP):
            u = _results(up, p * 49, 49)
            g = [[_gelu(_add_rows(u[r][c], b1_s[:, c * QF + p * 128:c * QF + (p + 1) * 128])) for c in range(4)]
                 for r in range(4)]
            hidden.append([o.astype(bf16) for o in _operands(_A_TERMS, g)])
        if more:
            out_proj(b + 1)
        down = paced(lambda i: _mm(jnp.concatenate([ops[i] for ops in hidden], axis=1), _unpack(w2s[i])),
                     48, y_jobs() if more else [])
        return _add_rows(h + _join(_results(down, 0, 49)), b2_s[...]).astype(bf16)

    def body(b, _):
        slot = b & 1

        @pl.when(b >= 2)
        def _():
            out_copy(b - 2, slot).wait()

        out_v[slot] = block(b, True)
        out_copy(b, slot).start()

    lax.fori_loop(0, NB - 1, body, None)
    out_copy(NB - 3, (NB - 3) % 2).wait()
    out_v[(NB - 1) % 2] = block(NB - 1, False)
    out_copy(NB - 1, (NB - 1) % 2).start()
    out_copy(NB - 2, (NB - 2) % 2).wait()
    out_copy(NB - 1, (NB - 1) % 2).wait()


def _kernel(x_hbm, wqkv_hbm, wo_hbm, w1_hbm, b1_hbm, w2_hbm, b2_hbm, out_hbm,
            x_v, b1_s, b2_s, wos, w1s, w2s, oT_s, h_s, t_s, oa_s, ya_s, zero_s, sem_x, sem_w, sem_p, sem_l, sem_out):
    def set_zero(i, _):
        zero_s[0] = i >> 10

    lax.fori_loop(0, 2, set_zero, None)
    mlp_input = _mlp_input(x_v, wos, oT_s, h_s, t_s, oa_s, ya_s)

    def through_attention(wo_v, b1_v, b2_v, k_s, qT_s, vT_s):
        late_copies = [pltpu.make_async_copy(src, dst, sem_l.at[n]) for n, (src, dst) in enumerate(
            [(b1_hbm, b1_v), (b2_hbm, b2_v), (wo_hbm, wo_v.at[pl.ds(0, D)])])]
        pl.run_scoped(
            functools.partial(_qkv_phase, x_hbm, wqkv_hbm, w1_hbm, w2_hbm, x_v, w1s, w2s, k_s, qT_s, vT_s, zero_s,
                              sem_x, sem_w, sem_p, late_copies),
            VMEM((D + 16, 3 * D), bf16), VMEM((7, HD // 2, 3 * HD), u32), VMEM((7, T // 2, HD), bf16),
            VMEM((1, T + 8, D), f32), VMEM((NP, 4, D + 16, 128), bf16), VMEM((NP, 4, 128 + 16, D), bf16))
        for c in late_copies:
            c.wait()
        b1_s[...] = jnp.broadcast_to(b1_v[...].astype(f32).reshape(1, F), (8, F))
        b2_s[...] = jnp.broadcast_to(b2_v[...].astype(f32).reshape(1, D), (8, D))
        pl.run_scoped(
            functools.partial(_attention_phase, k_s, qT_s, vT_s, oT_s, wo_v, wos, zero_s, mlp_input),
            *([VMEM((1, S, T), f32)] * NSB))

    pl.run_scoped(through_attention, VMEM((D + 16, D), bf16), VMEM((F,), bf16), VMEM((D,), bf16),
                  VMEM((G, S, 128), bf16), VMEM((NB, D, T), bf16), VMEM((NB, D, T), bf16))
    pl.run_scoped(
        functools.partial(_mlp_phase, out_hbm, b1_s, b2_s, w1s, w2s, h_s, ya_s, sem_out, mlp_input),
        VMEM((2, T, D), bf16))


@jax.jit
def pallas_sequential_preLN__softmax_full_mha__mixer_channel_mlp__prompt_kernel(
    A_x: jax.Array,
    A_wqkv: jax.Array,
    A_wo: jax.Array,
    B_x: jax.Array,
    B_w1: jax.Array,
    B_b1: jax.Array,
    B_w2: jax.Array,
    B_b2: jax.Array,
):
    del B_x
    hbm = pl.BlockSpec(memory_space=pl.ANY)
    out = pl.pallas_call(
        _kernel,
        name="fused",
        out_shape=jax.ShapeDtypeStruct((S, D), bf16),
        in_specs=[hbm] * 7,
        out_specs=hbm,
        scratch_shapes=[
            VMEM((S + 16, D), bf16), VMEM((8, F), f32), VMEM((8, D), f32),
            VMEM((49, QD // 2, QD), u32), VMEM((49, NP, QD // 2, 128), u32), VMEM((49, QF // 2, QD), u32),
            VMEM((NB + 1, D, T), bf16), VMEM((1, T + 8, D), f32), VMEM((1, T + 8, D), f32),
            VMEM((49, QT, QD), bf16), VMEM((49, QT, QD), bf16),
            pltpu.SMEM((1,), jnp.int32),
            pltpu.SemaphoreType.DMA((NB,)), pltpu.SemaphoreType.DMA((len(W_CHUNKS),)),
            pltpu.SemaphoreType.DMA((NP,)), pltpu.SemaphoreType.DMA((3,)), pltpu.SemaphoreType.DMA((2,)),
        ],
        compiler_params=pltpu.CompilerParams(vmem_limit_bytes=127 * 1024 * 1024),
    )(A_x.reshape(S, D), A_wqkv, A_wo, B_w1, B_b1, B_w2, B_b2)
    return out.reshape(1, S, D)
```

```python
import functools

import jax
import jax.numpy as jnp
import numpy as np
from jax import lax
from jax.experimental import pallas as pl
from jax.experimental.pallas import tpu as pltpu

S, D, H, DH, F = 2048, 1024, 32, 32, 3584
EPS = 1e-5
Q_SCALE = float(DH ** -0.5 * np.log2(np.e))
GELU_C0 = float(np.sqrt(2.0 / np.pi))
GELU_C1 = GELU_C0 * 0.044715

T = 256
NB = S // T
G = D // 128
HPG = 128 // DH
CK = 128
NC = S // CK
NH = NB * H
U = 24
NU = 10
LAG = 4
WO_EARLY = 3
NSB = 4
HD = D // 2
QT, QD, QF = T // 4, D // 4, F // 4
NP = QF // 128
W_CHUNKS = (256, 256, 256, 256, 512, 512, 512, 512)
W_ORDER = (0, 2 * D, D)
X1_CHUNK = 6
assert NP == NB - 1 and sum(W_CHUNKS) == 3 * D

f32, bf16, u32 = jnp.float32, jnp.bfloat16, jnp.uint32
VMEM = pltpu.VMEM


def _layernorm(x):
    xc = x - jnp.mean(x, axis=-1, keepdims=True)
    return xc * lax.rsqrt(jnp.mean(xc * xc, axis=-1, keepdims=True) + EPS)


def _gelu(u):
    hu = 0.5 * u
    return hu + hu * jnp.tanh(u * (GELU_C0 + GELU_C1 * (u * u)))


def _mm(a, b):
    return jnp.dot(a, b, preferred_element_type=f32)


def _times(i, n):
    return i * n if isinstance(i, int) else pl.multiple_of(i * n, n)


def _add_rows(x, row):
    return (x.reshape(x.shape[0] // 8, 8, x.shape[1]) + row[None]).reshape(x.shape)


def _pack(x):
    return pltpu.bitcast(x.astype(bf16), u32)


def _unpack(x):
    return pltpu.bitcast(x, bf16)


_A_TERMS = (((0, 0, 1), (1, 1, 1)), ((1, 0, 1), (1, 1, 1)), ((0, 0, 1),), ((1, 1, 1),),
            ((0, 0, 1), (0, 1, 1)), ((1, 0, 1), (0, 0, -1)), ((0, 1, 1), (1, 1, -1)))
_B_TERMS = (((0, 0, 1), (1, 1, 1)), ((0, 0, 1),), ((0, 1, 1), (1, 1, -1)), ((1, 0, 1), (0, 0, -1)),
            ((1, 1, 1),), ((0, 0, 1), (0, 1, 1)), ((1, 0, 1), (1, 1, 1)))


def _add(a, b):
    return [[p + q for p, q in zip(ra, rb)] for ra, rb in zip(a, b)]


def _sub(a, b):
    return [[p - q for p, q in zip(ra, rb)] for ra, rb in zip(a, b)]


def _combine(terms, quadrant):
    acc = None
    for rh, ch, sign in terms:
        q = quadrant(rh, ch)
        acc = q if acc is None else (_add if sign > 0 else _sub)(acc, q)
    return acc


def _operands(all_terms, x):
    if len(x) == 1:
        return [x[0][0]]
    n = len(x) // 2
    quadrant = lambda rh, ch: [row[ch * n:(ch + 1) * n] for row in x[rh * n:(rh + 1) * n]]
    return [o for terms in all_terms for o in _operands(all_terms, _combine(terms, quadrant))]


def _results(product, first, n):
    if n == 1:
        return [[product(first)]]
    m1, m2, m3, m4, m5, m6, m7 = [_results(product, first + i * (n // 7), n // 7) for i in range(7)]
    c11 = _add(_sub(_add(m1, m4), m5), m7)
    c12 = _add(m3, m5)
    c21 = _add(m2, m4)
    c22 = _add(_add(_sub(m1, m2), m3), m6)
    return [a + b for a, b in zip(c11, c12)] + [a + b for a, b in zip(c21, c22)]


def _join(grid):
    return jnp.concatenate([jnp.concatenate(row, axis=1) for row in grid], axis=0)


def _second_level(all_terms, load, store, i1):
    quadrant = lambda rh, ch: [[load(2 * rh + r, 2 * ch + c) for c in range(2)] for r in range(2)]
    for i2, o in enumerate(_operands(all_terms, _combine(all_terms[i1], quadrant))):
        store(i1 * 7 + i2, o)


def _park(ref, z, r):
    if len(ref.shape) == 2:
        ref[pl.ds(pl.multiple_of(ref.shape[0] - 16 + z * 16, 16), 16), :128] = r[:16, :128].astype(bf16)
    elif len(ref.shape) == 4:
        ref[z, 0, ref.shape[2] - 16:, :128] = r[:16, :128].astype(bf16)
    elif ref.dtype == f32:
        ref[z, ref.shape[1] - 8:, :128] = r[:8, :128]
    else:
        ref[ref.shape[0] - 1 + z, :16, :128] = r[:16, :128].astype(bf16)


def _spread(r, jobs, z):
    row_tiles = r.shape[0] // 16
    tiles = row_tiles * (r.shape[1] // 128)
    for e, (ref, fn) in enumerate(jobs):
        j, a = divmod(e * tiles // len(jobs), row_tiles)
        _park(ref, z, r[a * 16:(a + 1) * 16, j * 128:(j + 1) * 128])
        fn()


def _interleave(few, many):
    if len(few) > len(many):
        few, many = many, few
    step = len(many) // len(few)
    return [t for e, job in enumerate(few) for t in [job] + many[e * step:(e + 1) * step]] + many[len(few) * step:]


def _qkv_phase(x_hbm, wqkv_hbm, w1_hbm, w2_hbm, x_v, w1s, w2s, k_s, qT_s, vT_s, zero_s, sem_x, sem_w, sem_p,
               late_copies, wqkv_v, wqs, xa_s, y_s, w1_v, w2_v):
    bounds = [sum(W_CHUNKS[:j]) for j in range(len(W_CHUNKS) + 1)]

    def x_copy(b):
        return pltpu.make_async_copy(x_hbm.at[pl.ds(b * T, T)], x_v.at[pl.ds(b * T, T)], sem_x.at[b])

    def w_col(j):
        return W_ORDER[bounds[j] // D] + bounds[j] % D

    def w_copy(j):
        cols = pl.ds(w_col(j), W_CHUNKS[j])
        return pltpu.make_async_copy(wqkv_hbm.at[:, cols], wqkv_v.at[pl.ds(0, D), cols], sem_w.at[j])

    def part_copies(p):
        c = _times(p, 128)
        return ([pltpu.make_async_copy(w1_hbm.at[:, pl.ds(n * QF + c, 128)], w1_v.at[p, n, pl.ds(0, D)], sem_p.at[p])
                 for n in range(4)]
                + [pltpu.make_async_copy(w2_hbm.at[pl.ds(n * QF + c, 128)], w2_v.at[p, n, pl.ds(0, 128)], sem_p.at[p])
                   for n in range(4)])

    queue = ([[x_copy(0)]]
             + [[w_copy(j)] + ([x_copy(1)] if j == X1_CHUNK else []) for j in range(len(W_CHUNKS))]
             + [[x_copy(2)], part_copies(0)])

    def advance(n):
        for _ in range(min(n, len(queue))):
            for c in queue.pop(0):
                c.start()

    def x_jobs(b):
        def norm(rg):
            rows = x_v[pl.ds(_times(b * (T // 16) + rg, 16), 16), :]
            y_s[0, rg * 16:(rg + 1) * 16, :] = _layernorm(rows.astype(f32))

        def encode(rg, j):
            grid = [[y_s[0, r * (T // 2) + rg * 16:r * (T // 2) + (rg + 1) * 16, c * HD + j * 128:c * HD + (j + 1) * 128]
                     for c in range(2)] for r in range(2)]
            for i, o in enumerate(_operands(_A_TERMS, grid)):
                xa_s[i, rg * 16:(rg + 1) * 16, j * 128:(j + 1) * 128] = o.astype(bf16)

        return ([(x_v, functools.partial(norm, rg)) for rg in range(T // 16)]
                + [(y_s, functools.partial(encode, rg, j)) for rg in range(T // 32) for j in range(HD // 128)])

    def wqkv_jobs(m):
        def encode(rg, j):
            grid = [[wqkv_v[r * HD + rg * 16:r * HD + (rg + 1) * 16,
                            W_ORDER[m] + c * HD + j * 128:W_ORDER[m] + c * HD + (j + 1) * 128].astype(f32)
                     for c in range(2)] for r in range(2)]
            for i, o in enumerate(_operands(_B_TERMS, grid)):
                wqs[i, rg * 8:(rg + 1) * 8, m * HD + j * 128:m * HD + (j + 1) * 128] = _pack(o)

        return [(wqkv_v, functools.partial(encode, rg, j)) for rg in range(HD // 16) for j in range(HD // 128)]

    def mlp_weight_jobs(p):
        jobs = []
        for rg in range(QD // 16):
            def load1(r, c, rg=rg):
                return w1_v[p, c, r * QD + rg * 16:r * QD + (rg + 1) * 16, :].astype(f32)

            def store1(i, o, rg=rg):
                w1s[i, p, rg * 8:(rg + 1) * 8, :] = _pack(o)

            jobs += [(w1_v, functools.partial(_second_level, _B_TERMS, load1, store1, i1)) for i1 in range(7)]
        for rg in range(128 // 16):
            for j in range(QD // 128):
                def load2(r, c, rg=rg, j=j):
                    return w2_v[p, r, rg * 16:(rg + 1) * 16, c * QD + j * 128:c * QD + (j + 1) * 128].astype(f32)

                def store2(i, o, rg=rg, j=j):
                    w2s[i, pl.ds(_times(p * 8 + rg, 8), 8), j * 128:(j + 1) * 128] = _pack(o)

                jobs += [(w2_v, functools.partial(_second_level, _B_TERMS, load2, store2, i1)) for i1 in range(7)]
        return jobs

    def put_q(b, q):
        qT_s[b] = (q * Q_SCALE).T.astype(bf16)

    def put_v(b, v):
        vT_s[b] = v.T.astype(bf16)

    def put_k(b, k):
        k = k.astype(bf16)
        for g in range(G):
            k_s[g, pl.ds(_times(b, T), T), :] = k[:, g * 128:(g + 1) * 128]

    puts = (put_q, put_v, put_k)

    advance(2)
    x_copy(0).wait()
    advance(2)
    y = _layernorm(x_v[:T, :].astype(f32)).astype(bf16)
    parts, deferred, backlog = [], [], []
    for j, width in enumerate(W_CHUNKS):
        last = j == len(W_CHUNKS) - 1
        w_copy(j).wait()
        advance(len(queue) if last else 1)
        if j == X1_CHUNK:
            x_copy(1).wait()
        lo = _mm(y[:, :HD], wqkv_v[:HD, w_col(j):w_col(j) + width])
        hi = _mm(y[:, HD:], wqkv_v[HD:D, w_col(j):w_col(j) + width])
        parts.append(lo + hi)
        for fn in deferred:
            fn()
        deferred = []
        if bounds[j + 1] % D == 0:
            m = bounds[j + 1] // D - 1
            deferred.append(functools.partial(puts[m], 0, jnp.concatenate(parts, axis=1)))
            parts = []
            backlog += wqkv_jobs(m)
        if j == X1_CHUNK:
            backlog = _interleave(x_jobs(1), backlog)
        n = len(backlog) if last else min(len(backlog), width * 3 // 16)
        z = zero_s[0]
        _spread(lo, backlog[:n * 5 // 9], z)
        _spread(hi[:, :width * 3 // 4 // 128 * 128], backlog[n * 5 // 9:n], z)
        backlog = backlog[n:]
    for fn in deferred:
        fn()

    def block(b, _):
        for c in part_copies(b - 1):
            c.wait()

        @pl.when(b + 1 < NB)
        def _():
            x_copy(b + 1).wait()
            for c in part_copies(b):
                c.start()

        @pl.when(b + 2 < NB)
        def _():
            x_copy(b + 2).start()

        @pl.when(b + 2 == NB)
        def _():
            for c in late_copies:
                c.start()

        xa = [xa_s[i] for i in range(7)]
        jobs = _interleave(x_jobs(jnp.minimum(b + 1, NB - 1)), mlp_weight_jobs(b - 1))
        per = -(-len(jobs) // 21)

        def product(i):
            r = _mm(xa[i % 7], _unpack(wqs[i % 7, :, i // 7 * HD:(i // 7 + 1) * HD]))
            _spread(r, jobs[i * per:(i + 1) * per], b >> 10)
            return r

        for m in range(3):
            puts[m](b, _join(_results(product, m * 7, 7)))

    lax.fori_loop(1, NB, block, None)


def _attention_phase(k_s, qT_s, vT_s, oT_s, wo_v, wos, zero_s, mlp_input, *score_bufs):
    def locate(pair):
        return pair >> 5, _times(pair & (H - 1), DH)

    def padded_q(pair, j):
        i, row = locate(pair)
        above = [jnp.zeros((j * DH, T), bf16)] if j > 0 else []
        below = [jnp.zeros(((HPG - 1 - j) * DH, T), bf16)] if j < HPG - 1 else []
        return jnp.concatenate(above + [qT_s[i, pl.ds(row, DH), :]] + below, axis=0)

    def fold(op, acc, x, order):
        for r in order:
            acc = x[r * 8:(r + 1) * 8] if acc is None else op(acc, x[r * 8:(r + 1) * 8])
        return acc

    def scores(pair, q, c, buf, m, z):
        s = _mm(k_s[(pair & (H - 1)) >> 2, c * CK:(c + 1) * CK, :], q)
        buf[z, c * CK:(c + 1) * CK, :] = s
        return fold(jnp.maximum, m, s, range(CK // 8)), s

    def weigh(pair, c, buf, m, denom, acc, z):
        s = buf[z, c * CK:(c + 1) * CK, :]
        p = jnp.exp2(s.reshape(CK // 8, 8, T) - m[None]).reshape(CK, T)
        denom = fold(jnp.add, denom, p, range(CK // 8 - 1, -1, -1))
        kb, kc = divmod(c, T // CK)
        pv = _mm(vT_s[kb, pl.ds(locate(pair)[1], DH), kc * CK:(kc + 1) * CK], p.astype(bf16))
        return denom, (pv if acc is None else acc + pv)

    def finish(pair, denom, acc):
        i, row = locate(pair)
        oT_s[i, pl.ds(row, DH), :] = (acc * (1.0 / jnp.sum(denom, axis=0, keepdims=True))).astype(bf16)

    def run(base, first, stop, m, ready, z_store, z_load, scores_stop, jobs=()):
        q = row_max = denom = acc = None
        for n in range(first, stop):
            done = None
            if n < scores_stop:
                h, c = divmod(n, NC)
                if q is None or c == 0:
                    q = padded_q(base + h, h % HPG)
                m, s = scores(base + h, q, c, score_bufs[h % NSB], None if c == 0 else m, z_store)
                if c == NC - 1:
                    done, m = jnp.broadcast_to(jnp.max(m, axis=0, keepdims=True), (8, T)), None
                for slot, ref, fn in jobs:
                    if slot == n - first:
                        if ref is not None:
                            _park(ref, z_store, s)
                        fn()
            if n >= NC + LAG:
                h, c = divmod(n - NC - LAG, NC)
                if c == 0:
                    row_max, denom, acc = ready, None, None
                denom, acc = weigh(base + h, c, score_bufs[h % NSB], row_max, denom, acc, z_load)
                if c == NC - 1:
                    finish(base + h, denom, acc)
            if done is not None:
                ready = done
        return m, ready

    def wo_jobs(rg):
        jobs = []
        for j in range(QD // 128):
            def load(r, c, j=j):
                rows = pl.ds(_times(r * (QD // 16) + rg, 16), 16)
                return wo_v[rows, c * QD + j * 128:c * QD + (j + 1) * 128].astype(f32)

            def store(i, o, j=j):
                wos[i, pl.ds(_times(rg, 8), 8), j * 128:(j + 1) * 128] = _pack(o)

            jobs += [(wo_v, functools.partial(_second_level, _B_TERMS, load, store, i1)) for i1 in range(7)]
        return jobs

    def pace(jobs, first, last):
        return [(first + e * (last - first) // len(jobs), ref, fn) for e, (ref, fn) in enumerate(jobs)]

    first, never, rest = NC + LAG, 1 << 30, NH - NU * U
    z = zero_s[0]
    early = [job for rg in range(NU, NU + WO_EARLY) for job in wo_jobs(rg)]
    state = run(0, 0, first, None, None, z, z + z, never, pace(early, 1, first))

    def body(t, state):
        return run(t * U, first, first + U * NC, *state, t >> 10, t >> 11, never, pace(wo_jobs(t), 4, U * NC - 4))

    state = lax.fori_loop(0, NU, body, state)

    o_jobs, out_proj, y_jobs = mlp_input
    jobs = (pace(_interleave(o_jobs(0), [job for rg in range(NU + WO_EARLY, QD // 16) for job in wo_jobs(rg)]), 2, 130)
            + [(130, None, functools.partial(out_proj, 0))] + pace(y_jobs(), 140, 235))
    z = zero_s[0]
    run(NH - rest, first, first + rest * NC, *state, z, z + z, rest * NC, jobs)


def _mlp_input(x_v, wos, oT_s, h_s, t_s, oa_s, ya_s):
    def encode_jobs(dst):
        jobs = []
        for i1 in range(7):
            for rg in range(QT // 16):
                for j in range(QD // 128):
                    def load(r, c, rg=rg, j=j):
                        return t_s[0, r * QT + rg * 16:r * QT + (rg + 1) * 16, c * QD + j * 128:c * QD + (j + 1) * 128]

                    def store(i, o, rg=rg, j=j):
                        dst[i, rg * 16:(rg + 1) * 16, j * 128:(j + 1) * 128] = o.astype(bf16)

                    jobs.append((t_s, functools.partial(_second_level, _A_TERMS, load, store, i1)))
        return jobs

    def o_jobs(b):
        def transpose(g, j):
            tile = oT_s[b, g * 128:(g + 1) * 128, j * 128:(j + 1) * 128]
            t_s[0, j * 128:(j + 1) * 128, g * 128:(g + 1) * 128] = tile.astype(f32).T

        return ([(oT_s, functools.partial(transpose, g, j)) for g in range(G) for j in range(T // 128)]
                + encode_jobs(oa_s))

    def out_proj(b):
        attn = _results(lambda i: _mm(oa_s[i], _unpack(wos[i])), 0, 49)
        for r in range(4):
            for c in range(4):
                x = x_v[pl.ds(_times(b * 4 + r, QT), QT), c * QD:(c + 1) * QD]
                h_s[0, r * QT:(r + 1) * QT, c * QD:(c + 1) * QD] = x.astype(f32) + attn[r][c]

    def y_jobs():
        def norm(rg):
            t_s[0, rg * 16:(rg + 1) * 16, :] = _layernorm(h_s[0, rg * 16:(rg + 1) * 16, :])

        return [(h_s, functools.partial(norm, rg)) for rg in range(T // 16)] + encode_jobs(ya_s)

    return o_jobs, out_proj, y_jobs


def _mlp_phase(out_hbm, b1_s, b2_s, w1s, w2s, h_s, ya_s, sem_out, mlp_input, out_v):
    o_jobs, out_proj, y_jobs = mlp_input

    def out_copy(b, slot):
        return pltpu.make_async_copy(out_v.at[slot], out_hbm.at[pl.ds(_times(b, T), T)], sem_out.at[slot])

    def block(b, more):
        def paced(product, n, jobs):
            def run(i):
                r = product(i)
                for e, (ref, fn) in enumerate(jobs):
                    if e * n // len(jobs) == i:
                        _park(ref, b >> 10, r)
                        fn()
                return r
            return run

        ya = [ya_s[i] for i in range(49)]
        h = h_s[0, :T]
        up = paced(lambda i: _mm(ya[i % 49], _unpack(w1s[i % 49, i // 49])), 49 * NP, o_jobs(b + 1) if more else [])
        hidden = []
        for p in range(NP):
            u = _results(up, p * 49, 49)
            g = [[_gelu(_add_rows(u[r][c], b1_s[:, c * QF + p * 128:c * QF + (p + 1) * 128])) for c in range(4)]
                 for r in range(4)]
            hidden.append([o.astype(bf16) for o in _operands(_A_TERMS, g)])
        if more:
            out_proj(b + 1)
        down = paced(lambda i: _mm(jnp.concatenate([ops[i] for ops in hidden], axis=1), _unpack(w2s[i])),
                     48, y_jobs() if more else [])
        return _add_rows(h + _join(_results(down, 0, 49)), b2_s[...]).astype(bf16)

    def body(b, _):
        slot = b & 1

        @pl.when(b >= 2)
        def _():
            out_copy(b - 2, slot).wait()

        out_v[slot] = block(b, True)
        out_copy(b, slot).start()

    lax.fori_loop(0, NB - 1, body, None)
    out_copy(NB - 3, (NB - 3) % 2).wait()
    out_v[(NB - 1) % 2] = block(NB - 1, False)
    out_copy(NB - 1, (NB - 1) % 2).start()
    out_copy(NB - 2, (NB - 2) % 2).wait()
    out_copy(NB - 1, (NB - 1) % 2).wait()


def _kernel(x_hbm, wqkv_hbm, wo_hbm, w1_hbm, b1_hbm, w2_hbm, b2_hbm, out_hbm,
            x_v, b1_s, b2_s, wos, w1s, w2s, oT_s, h_s, t_s, oa_s, ya_s, zero_s, sem_x, sem_w, sem_p, sem_l, sem_out):
    def set_zero(i, _):
        zero_s[0] = i >> 10

    lax.fori_loop(0, 2, set_zero, None)
    mlp_input = _mlp_input(x_v, wos, oT_s, h_s, t_s, oa_s, ya_s)

    def through_attention(wo_v, b1_v, b2_v, k_s, qT_s, vT_s):
        late_copies = [pltpu.make_async_copy(src, dst, sem_l.at[n]) for n, (src, dst) in enumerate(
            [(b1_hbm, b1_v), (b2_hbm, b2_v), (wo_hbm, wo_v.at[pl.ds(0, D)])])]
        pl.run_scoped(
            functools.partial(_qkv_phase, x_hbm, wqkv_hbm, w1_hbm, w2_hbm, x_v, w1s, w2s, k_s, qT_s, vT_s, zero_s,
                              sem_x, sem_w, sem_p, late_copies),
            VMEM((D + 16, 3 * D), bf16), VMEM((7, HD // 2, 3 * HD), u32), VMEM((7, T // 2, HD), bf16),
            VMEM((1, T + 8, D), f32), VMEM((NP, 4, D + 16, 128), bf16), VMEM((NP, 4, 128 + 16, D), bf16))
        for c in late_copies:
            c.wait()
        b1_s[...] = jnp.broadcast_to(b1_v[...].astype(f32).reshape(1, F), (8, F))
        b2_s[...] = jnp.broadcast_to(b2_v[...].astype(f32).reshape(1, D), (8, D))
        pl.run_scoped(
            functools.partial(_attention_phase, k_s, qT_s, vT_s, oT_s, wo_v, wos, zero_s, mlp_input),
            *([VMEM((1, S, T), f32)] * NSB))

    pl.run_scoped(through_attention, VMEM((D + 16, D), bf16), VMEM((F,), bf16), VMEM((D,), bf16),
                  VMEM((G, S, 128), bf16), VMEM((NB, D, T), bf16), VMEM((NB, D, T), bf16))
    pl.run_scoped(
        functools.partial(_mlp_phase, out_hbm, b1_s, b2_s, w1s, w2s, h_s, ya_s, sem_out, mlp_input),
        VMEM((2, T, D), bf16))


@jax.jit
def pallas_sequential_preLN__softmax_full_mha__mixer_channel_mlp__prompt_kernel(
    A_x: jax.Array,
    A_wqkv: jax.Array,
    A_wo: jax.Array,
    B_x: jax.Array,
    B_w1: jax.Array,
    B_b1: jax.Array,
    B_w2: jax.Array,
    B_b2: jax.Array,
):
    del B_x
    hbm = pl.BlockSpec(memory_space=pl.ANY)
    out = pl.pallas_call(
        _kernel,
        name="fused",
        out_shape=jax.ShapeDtypeStruct((S, D), bf16),
        in_specs=[hbm] * 7,
        out_specs=hbm,
        scratch_shapes=[
            VMEM((S + 16, D), bf16), VMEM((8, F), f32), VMEM((8, D), f32),
            VMEM((49, QD // 2, QD), u32), VMEM((49, NP, QD // 2, 128), u32), VMEM((49, QF // 2, QD), u32),
            VMEM((NB + 1, D, T), bf16), VMEM((1, T + 8, D), f32), VMEM((1, T + 8, D), f32),
            VMEM((49, QT, QD), bf16), VMEM((49, QT, QD), bf16),
            pltpu.SMEM((1,), jnp.int32),
            pltpu.SemaphoreType.DMA((NB,)), pltpu.SemaphoreType.DMA((len(W_CHUNKS),)),
            pltpu.SemaphoreType.DMA((NP,)), pltpu.SemaphoreType.DMA((3,)), pltpu.SemaphoreType.DMA((2,)),
        ],
        compiler_params=pltpu.CompilerParams(vmem_limit_bytes=124 * 1024 * 1024),
    )(A_x.reshape(S, D), A_wqkv, A_wo, B_w1, B_b1, B_w2, B_b2)
    return out.reshape(1, S, D)
```
